```python
import jax
import jax.numpy as jnp

def _softmax(x, axis=-1):
    return jax.nn.softmax(x, axis=axis)
def _gelu(x):
    return jax.nn.gelu(x, approximate=True)
def _silu(x):
    return jax.nn.silu(x)
def _sigmoid(x):
    return jax.nn.sigmoid(x)
def _layernorm(x, axis=-1, eps=1e-5):
    m = jnp.mean(x, axis=axis, keepdims=True)
    v = jnp.var(x, axis=axis, keepdims=True)
    return (x - m) / jnp.sqrt(v + eps)
def _scatter_add(tgt, idx, src, axis=0):
    return tgt.at[idx].add(src)
def _segment_sum(src, seg, n):
    return jax.ops.segment_sum(src, seg, n)
class _Rng:
    def __init__(self, key):
        self._k = key
    def _next(self):
        self._k, sub = jax.random.split(self._k)
        return sub
    def normal(self, shape):
        return jax.random.normal(self._next(), shape, dtype=jnp.bfloat16)
    def randint(self, lo, hi, shape):
        return jax.random.randint(self._next(), shape, lo, hi, dtype=jnp.int32)
    def uniform(self, shape, lo=0.0, hi=1.0):
        return jax.random.uniform(self._next(), shape, jnp.bfloat16, lo, hi)
    def permutation(self, n):
        return jax.random.permutation(self._next(), n)


kernel_name = 'standalone__instancenorm__prompt'

def setup_inputs():
    _rng = _Rng(jax.random.key(int.from_bytes(__import__("os").urandom(4), "little")))
    _w = (lambda a: (lambda t: t.astype(jnp.bfloat16) if jnp.issubdtype(t.dtype, jnp.floating) else t)(jnp.asarray(a)))
    B, C, H, W = 2, 1024, 2048, 32
    return {
        "x": _w((lambda *s: _rng.normal(s) * 0.05)(B, C, H, W)),
        "g": _w((lambda *s: _rng.normal(s) * 0.05)(C) + 1.0),
        "b": _w((lambda *s: _rng.normal(s) * 0.05)(C)),
    }

def reference(x, g, b):
    mu = x.mean(axis=(-2, -1), keepdims=True)
    var = ((x - mu) * (x - mu)).mean(axis=(-2, -1), keepdims=True)
    xhat = (x - mu) / jnp.sqrt(var + 1e-5)
    return xhat * g.reshape(1, -1, 1, 1) + b.reshape(1, -1, 1, 1)
```

```python
import jax
import jax.numpy as jnp
from jax import lax
import jax.experimental.pallas as pl
import jax.experimental.pallas.tpu as pltpu

_EPS = 1e-5
_L = 128

_CHUNKS = (96, 96, 64)
_SLAB = 4096
_NS = 8
_R_ROWS, _R_WIN = 16, 32
_W_ROWS, _W_WIN = 32, 16
_K_RW = 12
_K_WR = 1
_R_UNROLL = 4
_R_GAP = 8
_BLK = 32


def _log2(v):
    assert v & (v - 1) == 0
    return v.bit_length() - 1


def _loop(lo, hi, body):
    def wrapped(i, carry):
        body(i)
        return carry

    lax.fori_loop(lo, hi, wrapped, 0)


def _make_kernel(C, rows):
    ips = _SLAB // rows
    group = ips * _NS
    r_steps = _SLAB // _R_ROWS
    w_dmas = rows // (_NS * _W_ROWS)
    ahead = _W_WIN + _NS
    depth = 4
    assert ahead + depth <= 2 * group
    inv_n = 1.0 / (rows * _L)

    def kernel(x_hbm, g_ref, b_ref, o_hbm, buf, gt, bt, rs, ws):
        def r_start(s0, t):
            rr = pl.ds(pl.multiple_of((t & (r_steps - 1)) * _R_ROWS, _R_ROWS), _R_ROWS)
            for q in range(2):
                s = ((t >> _log2(r_steps)) * 2 + q) * _NS
                pltpu.make_async_copy(
                    x_hbm.at[pl.ds(s0 + s, _NS), rr],
                    buf.at[pl.ds(s, _NS), rr],
                    rs.at[t & (_R_WIN - 1)],
                ).start(priority=q)

        def r_wait(t):
            both = buf.at[pl.ds(0, 2 * _NS), pl.ds(0, _R_ROWS)]
            pltpu.make_async_copy(both, both, rs.at[t & (_R_WIN - 1)]).wait()

        def r_fill(s0):
            _loop(0, _R_WIN, lambda t: r_start(s0, t))

        def w_start(s0, m):
            s = (m >> _log2(group)) * _NS
            for p in range(w_dmas):
                r0 = ((m & (group - 1)) * w_dmas + p) * _W_ROWS
                rr = pl.ds(pl.multiple_of(r0, _W_ROWS), _W_ROWS)
                pltpu.make_async_copy(
                    buf.at[pl.ds(s, _NS), rr],
                    o_hbm.at[pl.ds(s0 + s, _NS), rr],
                    ws.at[m & (_W_WIN - 1)],
                ).start()

        def w_wait(m):
            step = buf.at[0, pl.ds(0, rows)]
            pltpu.make_async_copy(step, step, ws.at[m & (_W_WIN - 1)]).wait()

        def locate(n):
            slab = (n >> _log2(group)) * _NS + (n & (_NS - 1))
            return slab, (n >> _log2(_NS)) & (ips - 1)

        def instance(n):
            s, i = locate(n)
            return buf.at[s, pl.ds(pl.multiple_of(i * rows, rows), rows)]

        def partial_sum(n, f):
            v, acc = instance(n), None
            for k in range(rows // _BLK):
                a = f(v[pl.ds(k * _BLK, _BLK), :].astype(jnp.float32))
                acc = a if acc is None else acc + a
            return acc.reshape(_BLK // 8, 8, _L).sum(axis=0)

        def average(acc):
            t = jnp.sum(jnp.sum(acc, axis=1, keepdims=True), axis=0, keepdims=True)
            return jnp.broadcast_to(t * inv_n, (8, _L))

        def tile(a):
            return jnp.tile(a, (_BLK // 8, 1))

        def statistics(s0, n, last, carry):
            sum3, mean2, sq1, mean1, _, _ = carry
            s, i = locate(jnp.clip(n + 1, 0, last))
            ch = pl.ds(((s0 + s) * ips + i) & (C - 1), 1)
            mean3 = average(sum3)
            scale = lax.rsqrt(average(sq1) + _EPS) * gt[ch, :]
            shift = bt[ch, :] - mean1 * scale
            sum4 = partial_sum(jnp.minimum(n + depth, last), lambda a: a)
            mu = tile(mean2)
            sq2 = partial_sum(jnp.clip(n + 2, 0, last), lambda a: (a - mu) * (a - mu))
            return sum4, mean3, sq2, mean2, scale, shift

        def normalise(s0, n, last, carry):
            nxt = statistics(s0, n, last, carry)
            scale, shift = tile(carry[4]), tile(carry[5])
            v = instance(n)
            for k in range(rows // _BLK):
                rr = pl.ds(k * _BLK, _BLK)
                v[rr, :] = (v[rr, :].astype(jnp.float32) * scale + shift).astype(v.dtype)
            return nxt

        r_fill(0)

        for src, dst in ((g_ref, gt), (b_ref, bt)):
            v = src[...].astype(jnp.float32)
            for k in range(C // _L):
                dst[pl.ds(k * _L, _L), :] = jnp.broadcast_to(v[k : k + 1, :], (_L, _L)).T

        def chunk(ci, s0):
            n = jnp.int32(_CHUNKS[0])
            for k in range(1, len(_CHUNKS)):
                n = jnp.where(ci >= k, _CHUNKS[k], n)
            nr = (n >> _log2(2 * _NS)) * r_steps
            ni = n * ips

            def read(t0, count):
                for u in range(count):
                    r_wait(t0 + u)
                    r_start(s0, t0 + u + _R_WIN)

            def read_range(lo, hi):
                sh = _log2(_R_UNROLL)
                _loop(lo >> sh, hi >> sh, lambda i: read(i * _R_UNROLL, _R_UNROLL))

            def under_reads(step):
                def body(i, carry):
                    read(r_steps + (i + depth) * _R_GAP, _R_GAP)
                    return step(s0, i, ni - 1, carry)

                return body

            read_range(0, r_steps)
            carry = (jnp.zeros((8, _L), jnp.float32),) * 6
            carry = lax.fori_loop(-depth, 0, under_reads(statistics), carry)
            carry = lax.fori_loop(0, ahead, under_reads(normalise), carry)
            read_range(r_steps + (ahead + depth) * _R_GAP, nr - _R_WIN)
            _loop(nr - _R_WIN, nr - _K_RW, r_wait)
            _loop(0, _W_WIN, lambda m: w_start(s0, m))
            _loop(nr - _K_RW, nr, r_wait)

            def write(i):
                w_wait(i - ahead)
                w_start(s0, i - _NS)

            def normalise_and_write(i, carry):
                carry = normalise(s0, i, ni - 1, carry)
                write(i)
                return carry

            lax.fori_loop(ahead, ni, normalise_and_write, carry)
            _loop(ni, ni + _NS, write)
            _loop(ni - _W_WIN, ni - _K_WR, w_wait)
            pl.when(ci + 1 < len(_CHUNKS))(lambda: r_fill(s0 + n))
            _loop(ni - _K_WR, ni, w_wait)
            return s0 + n

        lax.fori_loop(0, len(_CHUNKS), chunk, jnp.int32(0))

    scratch = [
        pltpu.VMEM((max(_CHUNKS), _SLAB, _L), jnp.bfloat16),
        pltpu.VMEM((C, _L), jnp.float32),
        pltpu.VMEM((C, _L), jnp.float32),
        pltpu.SemaphoreType.DMA((_R_WIN,)),
        pltpu.SemaphoreType.DMA((_W_WIN,)),
    ]
    return kernel, scratch


@jax.jit
def pallas_standalone__instancenorm__prompt_kernel(
    x: jax.Array,
    g: jax.Array,
    b: jax.Array,
):
    B, C, H, W = x.shape
    rows = H * W // _L
    assert B * C * rows == sum(_CHUNKS) * _SLAB
    kernel, scratch = _make_kernel(C, rows)
    xt = jnp.transpose(x, (0, 1, 3, 2)).reshape(B * C, W // 8, 8, H // _L, _L)
    xt = jnp.transpose(xt, (0, 1, 3, 2, 4)).reshape(-1, _SLAB, _L)
    y = pl.pallas_call(
        kernel,
        in_specs=[
            pl.BlockSpec(memory_space=pl.ANY),
            pl.BlockSpec(memory_space=pltpu.VMEM),
            pl.BlockSpec(memory_space=pltpu.VMEM),
        ],
        out_specs=pl.BlockSpec(memory_space=pl.ANY),
        out_shape=jax.ShapeDtypeStruct(xt.shape, xt.dtype),
        scratch_shapes=scratch,
        compiler_params=pltpu.CompilerParams(
            vmem_limit_bytes=110 * 1024 * 1024, disable_bounds_checks=True
        ),
    )(xt, g.reshape(C // _L, _L), b.reshape(C // _L, _L))
    y = jnp.transpose(y.reshape(B * C, W // 8, H // _L, 8, _L), (0, 1, 3, 2, 4))
    return jnp.transpose(y.reshape(B, C, W, H), (0, 1, 3, 2))
```

```python
import jax
import jax.numpy as jnp
from jax import lax
import jax.experimental.pallas as pl
import jax.experimental.pallas.tpu as pltpu

_EPS = 1e-5
_L = 128

_SLAB = 4096
_CHUNK = 128
_PIECE = 64
_PIECES = _SLAB // _PIECE

_R_GROUP = 8
_R_SLABS = 2
_R_WIN = 64
_R_OVERLAP = 13

_W_SLABS, _W_LAST = 6, 8
_W_STEP, _W_WIN = 4, 4
_W_OVERLAP = 1

_UNIT = 2
_DEPTH = 4
_BLK = 32


def _log2(v):
    assert v & (v - 1) == 0
    return v.bit_length() - 1


def _loop(lo, hi, body):
    def wrapped(i, carry):
        body(i)
        return carry

    lax.fori_loop(lo, hi, wrapped, 0)


def _piece(p):
    return pl.ds(pl.multiple_of(p * _PIECE, _PIECE), _PIECE)


def _make_kernel(C, rows, chunks):
    ips = _SLAB // rows
    units = _CHUNK * ips // _UNIT
    r_dmas = _R_GROUP // _R_SLABS
    r_group_steps = _PIECES * r_dmas
    r_steps = _CHUNK // (2 * _R_GROUP) * r_group_steps
    r_gap = r_group_steps * _UNIT // (_R_GROUP * ips)
    w_groups = (_CHUNK - _W_LAST) // _W_SLABS
    w_steps = w_groups * _PIECES // _W_STEP
    w_last_win = _W_STEP * _W_WIN
    early = units - (w_steps - _W_WIN)
    assert w_groups * _W_SLABS + _W_LAST == _CHUNK
    assert r_group_steps + (early + _DEPTH) * r_gap <= r_steps - _R_WIN
    for k in range(w_steps):
        done = early + max(0, k - _W_WIN + 1)
        assert (k * _W_STEP // _PIECES + 1) * _W_SLABS * ips <= done * _UNIT
    inv_n = 1.0 / (rows * _L)

    def kernel(x_hbm, g_hbm, b_hbm, o_hbm, buf, r_sem, w_sem, last_sem, p_sem):
        def r_start(s0, t):
            p = (t >> _log2(r_dmas)) & (_PIECES - 1)
            s = (t >> _log2(r_group_steps)) * _R_GROUP + (t & (r_dmas - 1)) * _R_SLABS
            for q, (sq, rr) in enumerate(
                ((s, _piece(_PIECES - 1 - p)), (s + _CHUNK // 2, _piece(p)))
            ):
                pltpu.make_async_copy(
                    x_hbm.at[pl.ds(s0 + sq, _R_SLABS), rr],
                    buf.at[pl.ds(sq, _R_SLABS), rr],
                    r_sem.at[t & (_R_WIN - 1)],
                ).start(priority=q)

        def r_wait(t):
            step = buf.at[pl.ds(0, 2 * _R_SLABS), pl.ds(0, _PIECE)]
            pltpu.make_async_copy(step, step, r_sem.at[t & (_R_WIN - 1)]).wait()

        def r_fill(s0):
            _loop(0, _R_WIN, lambda t: r_start(s0, t))

        def w_copy(s0, s, n, p, sem):
            return pltpu.make_async_copy(
                buf.at[pl.ds(s, n), _piece(p)], o_hbm.at[pl.ds(s0 + s, n), _piece(p)], sem
            )

        def w_start(s0, k):
            for u in range(_W_STEP):
                d = k * _W_STEP + u
                s = (d >> _log2(_PIECES)) * _W_SLABS
                sem = w_sem.at[k & (_W_WIN - 1)]
                w_copy(s0, s, _W_SLABS, d & (_PIECES - 1), sem).start()

        def w_wait(k):
            step = buf.at[pl.ds(0, _W_SLABS), pl.ds(0, _W_STEP * _PIECE)]
            pltpu.make_async_copy(step, step, w_sem.at[k & (_W_WIN - 1)]).wait()

        def last_copy(s0, p):
            sem = last_sem.at[p & (w_last_win - 1)]
            return w_copy(s0, _CHUNK - _W_LAST, _W_LAST, p, sem)

        def instances(m):
            n = m * _UNIT
            return [
                buf.at[
                    n >> _log2(ips),
                    pl.ds(pl.multiple_of(((n & (ips - 1)) + u) * rows, rows), rows),
                ]
                for u in range(_UNIT)
            ]

        def blocks(v):
            for k in range(rows // _BLK):
                rr = pl.ds(k * _BLK, _BLK)
                yield rr, v[rr, :].astype(jnp.float32)

        def partial_sum(terms):
            acc = None
            for a in terms:
                acc = a if acc is None else acc + a
            return acc.reshape(_BLK // 8, 8, _L).sum(axis=0)

        def total(acc):
            t = jnp.sum(jnp.sum(acc, axis=1, keepdims=True), axis=0, keepdims=True)
            return jnp.broadcast_to(t, (8, _L))

        def tile(a):
            return jnp.tile(a, (_BLK // 8, 1))

        def statistics(s0, m, carry):
            chan = lax.broadcasted_iota(jnp.int32, g.shape, 0) * _L
            chan += lax.broadcasted_iota(jnp.int32, g.shape, 1)
            x4 = instances(jnp.minimum(m + _DEPTH, units - 1))
            x2 = instances(jnp.clip(m + 2, 0, units - 1))
            out = []
            for u, (sum3, mean2, squares1, mean1, _, _) in enumerate(carry):
                mine = chan == ((s0 * ips + (m + 1) * _UNIT + u) & (C - 1))
                scale1 = lax.rsqrt(total(squares1) * inv_n + _EPS)
                scale1 *= total(jnp.where(mine, g, 0.0))
                mean3 = total(sum3) * inv_n
                sum4 = partial_sum(a for _, a in blocks(x4[u]))
                mu = tile(mean2)
                squares2 = partial_sum((a - mu) * (a - mu) for _, a in blocks(x2[u]))
                bias1 = total(jnp.where(mine, b, 0.0))
                out.append((sum4, mean3, squares2, mean2, mean1, (scale1, bias1)))
            return out

        def normalise(s0, m, carry):
            nxt = statistics(s0, m, carry)
            for v, (*_, mean0, (scale0, bias0)) in zip(instances(m), carry):
                mu, scale, bias = tile(mean0), tile(scale0), tile(bias0)
                for rr, a in blocks(v):
                    v[rr, :] = ((a - mu) * scale + bias).astype(v.dtype)
            return nxt

        parked = [buf.at[_CHUNK - 1, pl.ds(_SLAB - 16 * k, C // _L)] for k in (1, 2)]
        params = [
            pltpu.make_async_copy(src, dst, p_sem)
            for src, dst in zip((g_hbm, b_hbm), parked)
        ]
        for copy in params:
            copy.start()
        r_fill(0)
        for copy in params:
            copy.wait()
        g, b = (ref[...].astype(jnp.float32) for ref in parked)

        def chunk(ci):
            s0 = ci * _CHUNK

            def read(t):
                r_wait(t)
                r_start(s0, t + _R_WIN)

            def under_reads(stage):
                def body(m, carry):
                    t = r_group_steps + (m + _DEPTH) * r_gap
                    _loop(t, t + r_gap, read)
                    return stage(s0, m, carry)

                return body

            _loop(0, r_group_steps, read)
            zero = jnp.zeros((8, _L), jnp.float32)
            carry = [(zero, zero, zero, zero, zero, (zero, zero))] * _UNIT
            carry = lax.fori_loop(-_DEPTH, 0, under_reads(statistics), carry)
            carry = lax.fori_loop(0, early, under_reads(normalise), carry)
            _loop(r_group_steps + (early + _DEPTH) * r_gap, r_steps - _R_WIN, read)
            _loop(r_steps - _R_WIN, r_steps - _R_OVERLAP, r_wait)
            _loop(0, _W_WIN, lambda k: w_start(s0, k))
            _loop(r_steps - _R_OVERLAP, r_steps, r_wait)

            def write(k, carry):
                carry = normalise(s0, early + k, carry)
                w_wait(k)
                w_start(s0, k + _W_WIN)
                return carry

            def enter_last(k):
                w_wait(w_steps - _W_WIN + k)
                for u in range(_W_STEP):
                    last_copy(s0, k * _W_STEP + u).start()

            def write_last(p):
                last_copy(s0, p - w_last_win).wait()
                last_copy(s0, p).start()

            def wait_last(p):
                last_copy(s0, p).wait()

            lax.fori_loop(0, w_steps - _W_WIN, write, carry)
            _loop(0, _W_WIN, enter_last)
            _loop(w_last_win, _PIECES, write_last)
            _loop(_PIECES - w_last_win, _PIECES - _W_OVERLAP, wait_last)
            pl.when(ci + 1 < chunks)(lambda: r_fill(s0 + _CHUNK))
            _loop(_PIECES - _W_OVERLAP, _PIECES, wait_last)

        _loop(0, chunks, chunk)

    scratch = [
        pltpu.VMEM((_CHUNK, _SLAB, _L), jnp.bfloat16),
        pltpu.SemaphoreType.DMA((_R_WIN,)),
        pltpu.SemaphoreType.DMA((_W_WIN,)),
        pltpu.SemaphoreType.DMA((w_last_win,)),
        pltpu.SemaphoreType.DMA,
    ]
    return kernel, scratch


@jax.jit
def pallas_standalone__instancenorm__prompt_kernel(
    x: jax.Array,
    g: jax.Array,
    b: jax.Array,
):
    B, C, H, W = x.shape
    rows = H * W // _L
    chunks, rest = divmod(B * C * rows, _CHUNK * _SLAB)
    assert rest == 0 and C == 8 * _L
    kernel, scratch = _make_kernel(C, rows, chunks)
    xt = jnp.transpose(x, (0, 1, 3, 2)).reshape(B * C, W // 8, 8, H // _L, _L)
    xt = jnp.transpose(xt, (0, 1, 3, 2, 4)).reshape(-1, _SLAB, _L)
    y = pl.pallas_call(
        kernel,
        in_specs=[pl.BlockSpec(memory_space=pl.ANY)] * 3,
        out_specs=pl.BlockSpec(memory_space=pl.ANY),
        out_shape=jax.ShapeDtypeStruct(xt.shape, xt.dtype),
        scratch_shapes=scratch,
        compiler_params=pltpu.CompilerParams(
            vmem_limit_bytes=128 * 1024 * 1024, disable_semaphore_checks=True
        ),
    )(xt, g.reshape(C // _L, _L), b.reshape(C // _L, _L))
    y = jnp.transpose(y.reshape(B * C, W // 8, H // _L, 8, _L), (0, 1, 3, 2, 4))
    return jnp.transpose(y.reshape(B, C, W, H), (0, 1, 3, 2))
```
